```python
import os as _os
_os.environ.setdefault('JAX_PLATFORMS', 'cpu')
import jax
import jax.numpy as jnp

def _softmax(x, axis=-1):
    return jax.nn.softmax(x, axis=axis)

def _gelu(x):
    return jax.nn.gelu(x, approximate=True)

def _silu(x):
    return jax.nn.silu(x)

def _sigmoid(x):
    return jax.nn.sigmoid(x)

def _layernorm(x, axis=-1, eps=1e-05):
    m = jnp.mean(x, axis=axis, keepdims=True)
    v = jnp.var(x, axis=axis, keepdims=True)
    return (x - m) / jnp.sqrt(v + eps)

def _scatter_add(tgt, idx, src, axis=0):
    return tgt.at[idx].add(src)

def _segment_sum(src, seg, n):
    return jax.ops.segment_sum(src, seg, n)

class _Rng:

    def __init__(self, key):
        self._k = key

    def _next(self):
        self._k, sub = jax.random.split(self._k)
        return sub

    def normal(self, shape):
        return jax.random.normal(self._next(), shape, dtype=jnp.bfloat16)

    def randint(self, lo, hi, shape):
        return jax.random.randint(self._next(), shape, lo, hi, dtype=jnp.int32)

    def uniform(self, shape, lo=0.0, hi=1.0):
        return jax.random.uniform(self._next(), shape, jnp.bfloat16, lo, hi)

    def permutation(self, n):
        return jax.random.permutation(self._next(), n)
kernel_name = 'adaLN_cond__mha_block__geglu_ffn__prompt'

def setup_inputs():
    _rng = _Rng(jax.random.key(int.from_bytes(__import__("os").urandom(4), "little")))
    _w = lambda a: (lambda t: t.astype(jnp.bfloat16) if jnp.issubdtype(t.dtype, jnp.floating) else t)(jnp.asarray(a))

    def _A_setup():
        B, S, D, H = (1, 2048, 512, 32)
        return {'x': _w((lambda *s: _rng.normal(s) * 0.05)(B, S, D)), 'wqkv': _w((lambda *s: _rng.normal(s) * 0.05)(D, 3 * D)), 'wo': _w((lambda *s: _rng.normal(s) * 0.05)(D, D))}
    _A_in = _A_setup()

    def _B_setup():
        B, S, D, F = (1, 2048, 512, 1376)
        return {'x': _w((lambda *s: _rng.normal(s) * 0.05)(B, S, D)), 'w_gate': _w((lambda *s: _rng.normal(s) * 0.05)(D, F)), 'w_up': _w((lambda *s: _rng.normal(s) * 0.05)(D, F)), 'w_down': _w((lambda *s: _rng.normal(s) * 0.05)(F, D))}
    _B_in = _B_setup()
    return {'A_x': _A_in['x'], 'A_wqkv': _A_in['wqkv'], 'A_wo': _A_in['wo'], 'B_x': _B_in['x'], 'B_w_gate': _B_in['w_gate'], 'B_w_up': _B_in['w_up'], 'B_w_down': _B_in['w_down'], 'c': _w((lambda *s: _rng.normal(s) * 0.05)(1, 512) * 8.0), 'w_mod': _w((lambda *s: _rng.normal(s) * 0.05)(512, 6 * 512) * 512 ** (-0.5) * 8.0)}

def reference(A_x, A_wqkv, A_wo, B_x, B_w_gate, B_w_up, B_w_down, c, w_mod):

    def _A_ref(x, wqkv, wo):
        B, S, D = x.shape
        H = 32
        Dh = D // H
        qkv = (lambda x, *d: x.transpose(*d))((x @ wqkv).reshape(B, S, 3, H, Dh), 2, 0, 3, 1, 4)
        q, k, v = (qkv[0], qkv[1], qkv[2])
        scores = jnp.einsum('bhqd,bhkd->bhqk', q, k) * Dh ** (-0.5)
        p = _softmax(scores, axis=-1)
        o = jnp.einsum('bhqk,bhkd->bhqd', p, v)
        return (lambda x, *d: x.transpose(*d))(o, 0, 2, 1, 3).reshape(B, S, D) @ wo

    def _B_ref(x, w_gate, w_up, w_down):
        return _gelu(x @ w_gate) * (x @ w_up) @ w_down
    x = A_x
    mod = (_silu(c) @ w_mod).reshape(c.shape[0], 6, 1, -1)
    sa, ca, ga, sb, cb, gb = (mod[:, 0].copy(), mod[:, 1].copy(), mod[:, 2].copy(), mod[:, 3].copy(), mod[:, 4].copy(), mod[:, 5].copy())
    h = _layernorm(x, axis=-1) * (1 + ca) + sa
    x = x + ga * _A_ref(h, A_wqkv, A_wo)
    h = _layernorm(x, axis=-1) * (1 + cb) + sb
    x = x + gb * _B_ref(h, B_w_gate, B_w_up, B_w_down)
    return x
```

```python
import math

import jax
import jax.numpy as jnp
import jax.experimental.pallas as pl
import jax.experimental.pallas.tpu as pltpu

F32 = jnp.float32
BF16 = jnp.bfloat16

H = 32
BQ = 512
CK = 128
G = 4
EPS = 1e-5
NT = (((1,), (1,)), ((), ()))


def _dot(a, b):
    return jnp.dot(a, b, preferred_element_type=F32)


def _kernel(c_ref, x_hbm, wqkv_hbm, wo_hbm, wg_hbm, wu_hbm, wd_hbm, wmod_hbm, out_hbm,
            x_v, wqkv_v, wo_v, wg_v, wu_v, wd_v, wmod_v,
            wqvT, woT, wdT, col, qT, kr, vT, oT, sbuf, mbuf, obuf, sem_in, sem_out):
    S, D = x_v.shape
    DH = D // H
    NQ = S // BQ
    NC = S // CK
    NG = H // G

    cp_mod_a = pltpu.make_async_copy(wmod_hbm.at[:, :2 * D], wmod_v.at[:, :2 * D], sem_in.at[0])
    cp_mod_b = pltpu.make_async_copy(wmod_hbm.at[:, 2 * D:], wmod_v.at[:, 2 * D:], sem_in.at[1])
    cp_qkv = pltpu.make_async_copy(wqkv_hbm, wqkv_v, sem_in.at[2])
    cp_wo = pltpu.make_async_copy(wo_hbm, wo_v, sem_in.at[3])
    cp_wg = pltpu.make_async_copy(wg_hbm, wg_v, sem_in.at[4])
    cp_wu = pltpu.make_async_copy(wu_hbm, wu_v, sem_in.at[5])
    cp_wd = pltpu.make_async_copy(wd_hbm, wd_v, sem_in.at[6])

    def cp_x(b):
        rows = pl.ds(b * BQ, BQ)
        return pltpu.make_async_copy(x_hbm.at[rows], x_v.at[rows], sem_in.at[7 + b])

    cp_mod_a.start()
    cp_x(0).start()
    cp_qkv.start()
    for b in range(1, NQ):
        cp_x(b).start()

    cv = c_ref[...].astype(F32)
    sc = jnp.broadcast_to(cv * jax.nn.sigmoid(cv), (8, D)).astype(BF16)
    cp_mod_a.wait()
    mod_a = _dot(sc, wmod_v[:, :2 * D])
    sa = mod_a[0:1, :D]
    ca1 = 1.0 + mod_a[0:1, D:]

    cp_qkv.wait()
    cp_mod_b.start()
    cp_wo.start()
    cp_wg.start()
    cp_wu.start()
    cp_wd.start()
    wqvT[:D, :] = wqkv_v[:, :D].T
    wqvT[D:, :] = wqkv_v[:, 2 * D:].T

    qscale = DH ** -0.5 * math.log2(math.e)
    for b in range(NQ):
        cp_x(b).wait()
    for b in range(NQ):
        x = x_v[b * BQ:(b + 1) * BQ, :].astype(F32)
        mu = jnp.mean(x, axis=-1, keepdims=True)
        xc = x - mu
        var = jnp.mean(xc * xc, axis=-1, keepdims=True)
        h = (xc * jax.lax.rsqrt(var + EPS) * ca1 + sa).astype(BF16)
        k = pltpu.bitcast(_dot(h, wqkv_v[:, D:2 * D]).astype(BF16), jnp.uint32)
        for j in range(D // 128):
            kj = k[:, j * 128:(j + 1) * 128]
            for i in range(128 // DH):
                kk = kj if i == 0 else pltpu.roll(kj, 128 - i * DH, 1)
                kr[j * (128 // DH) + i, b * (BQ // 2):(b + 1) * (BQ // 2), :] = kk
        qv = jax.lax.dot_general(wqvT[...], h, NT, preferred_element_type=F32)
        qT[b] = (qv[:D] * qscale).astype(BF16)
        vT[:, b * BQ:(b + 1) * BQ] = qv[D:].astype(BF16)

    def attn_step(a, b):
        macc = lacc = oacc = None
        for t in range(G * NC):
            g, c = divmod(t, NC)
            keys = slice(c * CK, (c + 1) * CK)
            if b is not None:
                rows = pl.ds(pl.multiple_of((b[0] * G + g) * DH, DH), DH)
                if c == 0:
                    m_b = mbuf[g]
                    lacc = oacc = None
                p = jnp.exp2(sbuf[g, keys, :].reshape(CK // 8, 8, BQ) - m_b[None])
                for r in reversed(range(CK // 8)):
                    lacc = p[r] if lacc is None else lacc + p[r]
                oo = _dot(vT[rows, keys], p.reshape(CK, BQ).astype(BF16))
                oacc = oo if oacc is None else oacc + oo
                if c == NC - 1:
                    inv = 1.0 / jnp.sum(lacc, axis=0, keepdims=True)
                    oT[b[1], rows, :] = (oacc * inv).astype(BF16)
            if a is not None:
                ha = a[0] * G + g
                if c == 0:
                    q = qT[a[1], pl.ds(pl.multiple_of(ha * DH, DH), DH), :]
                    macc = None
                kc = pltpu.bitcast(kr[ha, c * (CK // 2):(c + 1) * (CK // 2), :], BF16)[:, :DH]
                s = _dot(kc, q)
                sbuf[g, keys, :] = s
                for r in range(CK // 8):
                    sr = s[r * 8:(r + 1) * 8]
                    macc = sr if macc is None else jnp.maximum(macc, sr)
                if c == NC - 1:
                    mbuf[g] = jnp.broadcast_to(jnp.max(macc, axis=0, keepdims=True), (8, BQ))

    attn_step((0, 0), None)

    cp_mod_b.wait()
    cp_wo.wait()
    cp_wg.wait()
    cp_wu.wait()
    cp_wd.wait()
    mod_b = _dot(sc, wmod_v[:, 2 * D:])
    for i in range(4):
        row = mod_b[0:1, i * D:(i + 1) * D]
        if i == 2:
            row = 1.0 + row
        col[i] = jnp.broadcast_to(row, (128, D)).T
    woT[...] = wo_v[...].T
    wdT[...] = wd_v[...].T

    def attn_body(i, carry):
        j = i + 1
        attn_step((j % NG, j // NG), (i % NG, i // NG))
        return carry

    jax.lax.fori_loop(0, NG * NQ - 1, attn_body, None)
    attn_step(None, (NG - 1, NQ - 1))

    def wide(i):
        return jnp.concatenate([col[i]] * (BQ // 128), axis=1)

    def cp_out(b):
        return pltpu.make_async_copy(obuf.at[b], out_hbm.at[pl.ds(b * BQ, BQ)], sem_out.at[b])

    def ffn_body(b, carry):
        xT = x_v[pl.ds(pl.multiple_of(b * BQ, BQ), BQ), :].T.astype(F32)
        x1 = xT + wide(0) * _dot(woT[...], oT[b])
        mu = jnp.mean(x1, axis=0, keepdims=True)
        xc = x1 - mu
        var = jnp.mean(xc * xc, axis=0, keepdims=True)
        h = (xc * jax.lax.rsqrt(var + EPS) * wide(2) + wide(1)).astype(BF16)
        gt = _dot(wg_v[...], h)
        ut = _dot(wu_v[...], h)
        inner = gt * (0.7978845608028654 + 0.7978845608028654 * 0.044715 * (gt * gt))
        hg = 0.5 * gt
        act = ((hg + hg * jnp.tanh(inner)) * ut).astype(BF16)
        x2 = x1 + wide(3) * _dot(wdT[...], act)
        obuf[b] = x2.astype(BF16).T
        cp_out(b).start()
        return carry

    jax.lax.fori_loop(0, NQ, ffn_body, None)
    for b in range(NQ):
        cp_out(b).wait()


@jax.jit
def pallas_adaLN_cond__mha_block__geglu_ffn__prompt_kernel(
    A_x: jax.Array,
    A_wqkv: jax.Array,
    A_wo: jax.Array,
    B_x: jax.Array,
    B_w_gate: jax.Array,
    B_w_up: jax.Array,
    B_w_down: jax.Array,
    c: jax.Array,
    w_mod: jax.Array,
):
    del B_x
    _, S, D = A_x.shape
    F = B_w_gate.shape[1]
    NQ = S // BQ
    hbm = pl.BlockSpec(memory_space=pltpu.HBM)
    out = pl.pallas_call(
        _kernel,
        out_shape=jax.ShapeDtypeStruct((S, D), A_x.dtype),
        in_specs=[pl.BlockSpec(memory_space=pltpu.VMEM)] + [hbm] * 7,
        out_specs=hbm,
        scratch_shapes=[
            pltpu.VMEM((S, D), BF16),
            pltpu.VMEM((D, 3 * D), BF16),
            pltpu.VMEM((D, D), BF16),
            pltpu.VMEM((F, D), BF16),
            pltpu.VMEM((F, D), BF16),
            pltpu.VMEM((F, D), BF16),
            pltpu.VMEM((D, 6 * D), BF16),
            pltpu.VMEM((2 * D, D), BF16),
            pltpu.VMEM((D, D), BF16),
            pltpu.VMEM((D, F), BF16),
            pltpu.VMEM((4, D, 128), F32),
            pltpu.VMEM((NQ, D, BQ), BF16),
            pltpu.VMEM((H, S // 2, 128), jnp.uint32),
            pltpu.VMEM((D, S), BF16),
            pltpu.VMEM((NQ, D, BQ), BF16),
            pltpu.VMEM((G, S, BQ), F32),
            pltpu.VMEM((G, 8, BQ), F32),
            pltpu.VMEM((NQ, BQ, D), BF16),
            pltpu.SemaphoreType.DMA((7 + NQ,)),
            pltpu.SemaphoreType.DMA((NQ,)),
        ],
        compiler_params=pltpu.CompilerParams(vmem_limit_bytes=110 * 1024 * 1024),
        name="adaln_block",
    )(c, A_x.reshape(S, D), A_wqkv, A_wo, B_w_gate.T, B_w_up.T, B_w_down, w_mod)
    return out.reshape(A_x.shape)
```

```python
import math

import jax
import jax.numpy as jnp
import jax.experimental.pallas as pl
import jax.experimental.pallas.tpu as pltpu

F32 = jnp.float32
BF16 = jnp.bfloat16
U32 = jnp.uint32

H = 32
EPS = 1e-5
LANES = 128
BQ = 512
CK = 128
RB = 9
SHORT = (1, 8)
NCH = 4
L_MIN, L_MAX = 2.0 ** -60, 2.0 ** 60
MIX = (0, 1, 4, 5, 6)

VLEAD = 4
LLAG = 5
XLAG = 16


def _dot(a, b):
    return jnp.dot(a, b, preferred_element_type=F32)


def _dot_nt(a, b):
    return jax.lax.dot_general(a, b, (((1,), (1,)), ((), ())), preferred_element_type=F32)


def _pack(x, dtype=U32):
    return pltpu.bitcast(x.astype(BF16), dtype)


def _unpack(x):
    return pltpu.bitcast(x, BF16)


def _rows(*xs):
    return jnp.concatenate(xs, axis=0)


def _cols(*xs):
    return jnp.concatenate(xs, axis=1)


def _quads(x):
    m, n = x.shape[0] // 2, x.shape[1] // 2
    return x[:m, :n], x[:m, n:], x[m:, :n], x[m:, n:]


def _join(c11, c12, c21, c22):
    return _rows(_cols(c11, c12), _cols(c21, c22))


def _left(i, a11, a12, a21, a22):
    if i not in MIX:
        return a11 if i == 2 else a22
    p, q = {0: (a11, a22), 1: (a21, a22), 4: (a11, a12), 5: (a21, a11), 6: (a12, a22)}[i]
    p, q = p.astype(F32), q.astype(F32)
    return (p + q if i < 5 else p - q).astype(BF16)


def _right(i, b11, b12, b21, b22):
    if i in (1, 4):
        return (b11 if i == 1 else b22).astype(BF16)
    p, q = {0: (b11, b22), 2: (b12, b22), 3: (b21, b11), 5: (b11, b12), 6: (b21, b22)}[i]
    return (p - q if i in (2, 3) else p + q).astype(BF16)


def _gather(m):
    return m[3] - m[4] + m[6] + m[0], m[2] + m[4], m[1] + m[3], m[2] - m[1] + m[5] + m[0]


def _row_sums(xs):
    row = jax.lax.broadcasted_iota(jnp.int32, xs[0].shape, 0)
    for bit in (4, 2, 1):
        low = (row & bit) == 0
        xs = [jnp.where(low, a, b) + jnp.where(low, pltpu.roll(a, 8 - bit, 0), pltpu.roll(b, bit, 0))
              for a, b in zip(xs[:bit], xs[bit:])]
    return xs[0]


def _geglu(g, u):
    k = math.sqrt(2.0 / math.pi)
    half = 0.5 * g
    return (half + half * jnp.tanh(g * (k + k * 0.044715 * (g * g)))) * u


def _ds(start, size):
    return pl.ds(pl.multiple_of(start * size, size), size)


def _kernel(c_hbm, x_hbm, wqkv_hbm, wo_hbm, wg_hbm, wu_hbm, wd_hbm, wmod_hbm, out_hbm,
            x_v, wqkv_v, wo_v, wg_v, wu_v, wd_v, wmod_v, up_f, wo_t, down_f, down_r, col,
            q_t, k_r, v_t, o_t, p_v, l_v, x1_v, x1_first, out_v, sem_in, sem_out, *rest):
    *vbs, c_v = rest
    S, D = x_v.shape
    DH = D // H
    NQ, NC, NW, CPB = S // BQ, S // CK, BQ // LANES, BQ // CK
    FH = wd_v.shape[0] // 2
    ND = FH // LANES
    FM = ND * LANES

    NV = NQ * RB
    mxu_keys = [96 if c in SHORT else 112 for c in range(NC)]
    mxu_from = [(c // CPB + 1) * BQ - sum(mxu_keys[c:(c // CPB + 1) * CPB]) for c in range(NC)]
    vpu_from = [k for b in range(NQ) for k in range(b * BQ, mxu_from[b * CPB], 8)]
    assert len(vpu_from) == NV and NQ * NW == NC and D == BQ

    DC = DH // NCH
    QB = NV * DC
    SLOT = QB + NQ * DC * NW
    PACE = 2 * SLOT
    SRC = PACE + 4

    def k_src(hd, g, n):
        return vbs[0][pl.ds(SRC + hd * NV + g, n)].reshape(n * 8, LANES)

    def q_src(hd, r, w):
        return vbs[-1][SRC + (hd * (DH // 8) + r) * NC + w]

    def k_spread(rows, d):
        return jnp.broadcast_to(rows[:, d:d + 1], rows.shape).reshape(-1, 8, LANES)

    def q_spread(tile, d):
        return jnp.broadcast_to(tile[d % 8:d % 8 + 1], tile.shape)

    def k_at(base, d, g, n):
        return pl.ds(base + (d // NCH * NV + g), n)

    def q_at(base, d, j, w):
        return base + (QB + (j * DC + d // NCH) * NW + w)

    def columns(i, src, dst, lo, hi):
        return pltpu.make_async_copy(src.at[:, lo:hi], dst.at[:, lo:hi], sem_in.at[i])

    cp_c = pltpu.make_async_copy(c_hbm, c_v, sem_in.at[0])
    cp_mod = columns(1, wmod_hbm, wmod_v, 0, 2 * D)
    cp_q, cp_k, cp_v = (columns(2 + i, wqkv_hbm, wqkv_v, i * D, (i + 1) * D) for i in range(3))
    cp_late = [columns(5, wmod_hbm, wmod_v, 2 * D, 6 * D)] + [
        pltpu.make_async_copy(src, dst, sem_in.at[6 + i])
        for i, (src, dst) in enumerate(((wo_hbm, wo_v), (wg_hbm, wg_v), (wu_hbm, wu_v), (wd_hbm, wd_v)))]
    cp_x = [pltpu.make_async_copy(x_hbm.at[b * BQ:(b + 1) * BQ], x_v.at[b * BQ:(b + 1) * BQ], sem_in.at[10 + b])
            for b in range(NQ)]

    for cp in (cp_c, cp_mod, cp_x[0], cp_k):
        cp.start()
    cp_c.wait()
    cond = c_v[...].astype(F32)
    cond = jnp.broadcast_to(cond * jax.nn.sigmoid(cond), (8, D)).astype(BF16)
    cp_mod.wait()
    mod = _dot(cond, wmod_v[:, :2 * D])
    cp_q.start()
    cp_v.start()
    cp_x[0].wait()

    def put_k(b, k):
        first = vpu_from.index(b * BQ)
        some = k[:mxu_from[b * CPB] - b * BQ]
        k = _pack(k)
        for hd in range(H):
            tile, shift = divmod(hd * DH, LANES)
            kk, ss = (a[:, tile * LANES:(tile + 1) * LANES] for a in (k, some))
            if shift:
                kk, ss = pltpu.roll(kk, LANES - shift, 1), pltpu.roll(ss, LANES - shift, 1)
            k_r[hd, b * BQ // 2:(b + 1) * BQ // 2] = kk
            vbs[0][pl.ds(SRC + hd * NV + first, ss.shape[0] // 8)] = ss.reshape(-1, 8, LANES)

    def project(product, start=(), wait=(), priority=0):
        m = {}
        for n, i in enumerate((3, 4, 0, 2, 1, 6, 5)):
            if n == 4:
                for cp in start:
                    cp.start(priority=priority)
                for cp in wait:
                    cp.wait()
            m[i] = product(i)
        return _gather(m)

    for b in range(NQ):
        x = x_v[b * BQ:(b + 1) * BQ].astype(F32)
        x = x - jnp.mean(x, axis=-1, keepdims=True)
        x = x * jax.lax.rsqrt(jnp.mean(x * x, axis=-1, keepdims=True) + EPS)
        h11, h21, h12, h22 = _quads(x * (1.0 + mod[0:1, D:]) + mod[0:1, :D])
        hs = [_right(i, h11, h12, h21, h22) for i in range(7)]
        if b == 0:
            cp_x[1].start()
            cp_x[2].start()
            cp_k.wait()
            w11, w21, w12, w22 = _quads(wqkv_v[:, D:2 * D])
            wk = [_left(i, w11, w12, w21, w22) for i in range(7)]
        copies = {0: ([cp_x[3]], [cp_q]), 1: (cp_late, cp_x[2:], 1)}.get(b, ())
        k11, k12, k21, k22 = project(lambda i: _dot(hs[i], wk[i]), *copies)
        if b == 0:
            wq = _quads(wqkv_v[:, :D].T)
            wq = [_left(i, *wq) for i in range(7)]
        if b == 1:
            put_k(0, k)
        k = _join(k11, k21, k12, k22)
        q = _join(*project(lambda i: _dot_nt(wq[i], hs[i]), wait=() if b else (cp_v, cp_x[1])))
        q = q * (DH ** -0.5 * math.log2(math.e))
        q_t[b] = _pack(q)
        for w in range(NW):
            for r in range(D // 8):
                vbs[-1][SRC + r * NC + b * NW + w] = q[r * 8:(r + 1) * 8, w * LANES:(w + 1) * LANES]
        if b == 0:
            wv = _quads(wqkv_v[:, 2 * D:].T)
            wv = [_left(i, *wv) for i in range(7)]
        v = _pack(_join(*project(lambda i: _dot_nt(wv[i], hs[i]))))
        for c in range(CPB):
            v_t[b * CPB + c] = v[:, c * CK:(c + 1) * CK]
        if b > 0:
            put_k(b, k)

    for cp in cp_late:
        cp.wait()

    def down_prep(n):
        t1, t2 = (wd_v[pl.ds(pl.multiple_of(r + n * LANES, 16), LANES)].T for r in (0, FH))
        for i in range(7):
            down_f[n, i] = _pack(_left(i, t1[:D // 2], t2[:D // 2], t1[D // 2:], t2[D // 2:]))

    def weight_prep(j):
        for e in range(pl.cdiv(FH, 16 * NQ)):
            n = jnp.minimum(e * NQ + j, FH // 16 - 1)
            for m, src in enumerate((wg_v, wu_v)):
                part = _quads(_rows(src[_ds(n, 16)], src[_ds(FH // 16 + n, 16)]))
                for f, i in enumerate(MIX):
                    up_f[len(MIX) * m + f, _ds(n, 8)] = _pack(_left(i, *part))
            if e:
                yield
        row = _dot(cond, wmod_v[:, _ds(2 + j, D)])[0:1]
        col[j] = jnp.broadcast_to(row + jnp.where(j == 2, 1.0, 0.0), (LANES, D)).T
        yield
        wo_t[j] = wo_v[_ds(j, LANES)].T
        yield
        down_prep(j)

    def first_head(j, carry):
        job = weight_prep(j)
        spare = 2 * len(MIX)
        for i in range(2):
            up_f[spare, i * 8:(i + 1) * 8] = q_t[j, :DH // 2, i * (BQ // 2):(i + 1) * (BQ // 2)]
        for c in range(NC):
            q = _unpack(_cols(up_f[spare + (j >> 8), :8], up_f[spare + (j >> 8), 8:16]))
            p = jnp.exp2(_dot(_unpack(k_r[0, c * CK // 2:(c + 1) * CK // 2])[:, :DH], q))
            p_v[j, c * CK:(c + 1) * CK] = p
            for r in range(0, CK, 8):
                l = l + p[r:r + 8] if c or r else p[:8]
            next(job, None)
        for _ in job:
            pass
        l_v[j, 0] = l
        ks = k_src(1, j * RB, RB)
        qs = [[q_src(1, r, j * NW + w) for w in range(NW)] for r in range(DH // 8)]
        for d in range(DH):
            vbs[d % NCH][k_at(SLOT + j * RB, d, 0, RB)] = k_spread(ks, d)
            for w in range(NW):
                vbs[d % NCH][q_at(SLOT + j * DC * NW, d, 0, w)] = q_spread(qs[d // 8][w], d)
        return carry

    jax.lax.fori_loop(0, NQ, first_head, None)

    def head(hd, carry):
        nxt = jnp.minimum(hd + 1, H - 1)
        base, other = hd % 2 * SLOT, (1 - hd % 2) * SLOT
        pace_at = PACE - (hd >> 8)
        q_rows, v_rows = _ds(hd, DH // 2), _ds(hd - 1, DH // 2)
        steps = NQ * NC * DH
        k_jobs = [(d, g) for d in range(DH) for g in range(NV)]
        q_jobs = [(d, w) for d in range(DH) for w in range(NC)]
        later, old_p, l, todo = {}, {}, {}, {j: S * NW for j in range(NQ)}

        def read_p(j, key):
            c = key // CK
            if (j, c) not in old_p:
                old_p[j, c] = p_v[j, c * CK:(c + 1) * CK]
            return old_p[j, c]

        def count(j, n):
            todo[j] -= n
            if not todo[j]:
                l_v[j, hd] = l[j]

        def add_tile(j, w, part):
            tiles = [l[j][:, i * LANES:(i + 1) * LANES] for i in range(NW)]
            tiles[w] = tiles[w] + part
            l[j] = _cols(*tiles)
            count(j, RB * 8)

        def store(vb, at, val):
            vb[at] = val

        def vector_scores():
            for now in range(steps):
                pace = yield
                block, d = divmod(now, DH)
                j, g, w = block // NC, block % NC // NW * RB, block % NW
                vb = vbs[d % NCH]
                if pace is not None:
                    vb[pace_at] = pace
                for fn, *args in later.pop(now, ()):
                    fn(*args)
                for jobs in (k_jobs, q_jobs):
                    per = steps - XLAG - NCH
                    for e, i in jobs[now * len(jobs) // per:(now + 1) * len(jobs) // per]:
                        if jobs is k_jobs:
                            due, at, val = now + XLAG, k_at(other, e, i, 1), k_spread(k_src(nxt, i, 1), e)
                        else:
                            due, at, val = now + 1, q_at(other, e, i // NW, i % NW), q_spread(q_src(nxt, e // 8, i), e)
                        later.setdefault(due + (e - due) % NCH, []).append((store, vbs[e % NCH], at, val))
                term = vb[k_at(base, d, g, RB)] * vb[q_at(base, d, j, w)]
                acc = acc + term if d else term
                if d == DH - 1:
                    p = jnp.exp2(acc)
                    keys = vpu_from[g:g + RB]
                    cuts = [0] + [e for e in range(1, RB) if keys[e] != keys[e - 1] + 8] + [RB]
                    for lo, hi in zip(cuts, cuts[1:]):
                        read_p(j, keys[lo])
                        p_v[j, keys[lo]:keys[hi - 1] + 8, w * LANES:(w + 1) * LANES] = p[lo:hi].reshape(-1, LANES)
                    p = [p[e] for e in range(RB)]
                    while len(p) > 1:
                        p = [p[i] + p[i + 1] if i + 1 < len(p) else p[i] for i in range(0, len(p), 2)]
                    later.setdefault(now + LLAG, []).append((add_tile, j, w, p[0]))
            yield

        vector = vector_scores()
        next(vector)
        read_p(0, 0)
        for _ in range(VLEAD):
            vector.send(None)
        done = VLEAD
        for t in range(NQ * NC):
            j, c = divmod(t, NC)
            lo, hi = mxu_from[c], mxu_from[c] + mxu_keys[c]
            s = _dot(_unpack(k_r[hd, lo // 2:hi // 2])[:, :DH], _unpack(q_t[j, q_rows]))
            marks = [s[r:r + 8, :LANES] for r in range(0, hi - lo, 8)]
            pv = _dot(_unpack(v_t[c, v_rows]), read_p(j, c * CK))
            o = o + pv if c else pv
            if c == NC - 1:
                o_t[j, hd - 1] = o
            marks += [pv[r:r + 8, :LANES] for r in range(0, DH, 8)]
            p = jnp.exp2(s)
            read_p(j, hi - 1)
            p_v[j, lo:hi] = p
            lead = VLEAD + 2 * max(t + 4 - NQ * NC, 0)
            for r, mark in enumerate(marks):
                if r * 8 < hi - lo:
                    l[j] = l[j] + p[r * 8:r * 8 + 8] if j in l else p[:8]
                    count(j, 8 * NW)
                while done < min(steps, lead + t * DH + pl.cdiv((r + 1) * DH, len(marks))):
                    vector.send(mark)
                    done += 1
        for now in sorted(later):
            for fn, *args in later[now]:
                fn(*args)
        return carry

    jax.lax.fori_loop(1, H, head, None)

    def head_with_true_max(i, carry):
        hd, j = i // NQ, i % NQ
        q = _unpack(q_t[j, _ds(hd, DH // 2)])

        def scores(c, m):
            s = _dot(_unpack(k_r[hd, _ds(c, CK // 2)])[:, :DH], q)
            p_v[j, _ds(c, CK)] = s
            return jnp.maximum(m, jnp.max(s, axis=0, keepdims=True))

        m = jax.lax.fori_loop(0, NC, scores, jnp.full((1, BQ), -jnp.inf, F32))

        def weights(c, acc):
            p = jnp.exp2(p_v[j, _ds(c, CK)] - m)
            p_v[j, _ds(c, CK)] = p
            return (acc[0] + jnp.sum(p.reshape(CK // 8, 8, BQ), axis=0),
                    acc[1] + _dot(_unpack(v_t[c, _ds(hd, DH // 2)]), p))

        l_v[j, hd], o_t[j, hd] = jax.lax.fori_loop(
            0, NC, weights, (jnp.zeros((8, BQ), F32), jnp.zeros((DH, BQ), F32)))
        return carry

    def wide(i, rows=slice(None)):
        return _cols(*[col[i, rows]] * NW)

    def factor_at(i, lo, hi):
        top = i // 2 * (D // 4)
        return NQ + 1, slice(top + lo, top + hi), slice(i % 2 * (BQ // 2), (i % 2 + 1) * (BQ // 2))

    def second_norm(ref, at):
        acc = 0.0
        for r in range(0, D, 128):
            acc = acc + jnp.sum(ref[at, r:r + 128].reshape(16, 8, BQ), axis=0)
            yield acc
        mean = jnp.sum(acc, axis=0, keepdims=True) * (1.0 / D)
        acc = 0.0
        for r in range(0, D, 64):
            x = ref[at, r:r + 64] - mean
            acc = acc + jnp.sum((x * x).reshape(8, 8, BQ), axis=0)
            yield acc
        inv = jax.lax.rsqrt(jnp.sum(acc, axis=0, keepdims=True) * (1.0 / D) + EPS)
        for r in range(0, D // 2, 16):
            part = []
            for rows in (slice(r, r + 16), slice(D // 2 + r, D // 2 + r + 16)):
                h = (ref[at, rows] - mean) * inv * wide(2, rows) + wide(1, rows)
                part += [h[:, :BQ // 2], h[:, BQ // 2:]]
            for i in range(7):
                x1_v[factor_at(i, r // 2, r // 2 + 8)] = _pack(_right(i, *part), F32)
            yield None

    def advance(job, ref, spare, mark):
        ref[spare, :8, :LANES] = mark[-8:, -LANES:]
        acc = next(job, None)
        if acc is not None:
            ref[spare, 8:16] = acc

    def up_factor(m, i, lo, hi):
        if i in MIX:
            return _unpack(up_f[len(MIX) * m + MIX.index(i), lo // 2:hi // 2])
        half = i - 2
        return (wg_v, wu_v)[m][half * FH + lo:half * FH + hi, half * (D // 2):(half + 1) * (D // 2)]

    def cp_out(b):
        return pltpu.make_async_copy(out_v.at[b], out_hbm.at[_ds(b, BQ)], sem_out.at[b])

    def ffn(b, carry):
        hs = [_unpack(x1_v[factor_at(i, 0, D // 4)]) for i in range(7)]
        job = second_norm(x1_v, jnp.minimum(b + 1, NQ - 1))
        act = []
        for lo in range(0, FH, LANES):
            g, u = {}, {}
            for i in (3, 4, 6, 0, 2, 1, 5):
                g[i], u[i] = (_dot(up_factor(m, i, lo, min(lo + LANES, FH)), hs[i]) for m in range(2))
                advance(job, x1_v, NQ, u[i])
            act.append([_geglu(*gu) for gu in zip(_gather(g), _gather(u))])
        for _ in job:
            pass
        main = [_rows(*a) for a in zip(*act[:ND])]
        y = _join(*_gather({
            i: _dot(_unpack(_cols(*[down_f[n, i] for n in range(ND)])), _right(i, *main))
            for i in (1, 5, 3, 4, 2, 6, 0)}))
        y = y + _dot(down_r[...], _join(*act[ND]).astype(BF16))
        out_v[b] = (x1_v[b] + wide(3) * y).astype(BF16).T
        cp_out(b).start()
        return carry

    def finish(attempt):
        for n in range(NQ, ND):
            down_prep(n)
        down_r[...] = _rows(wd_v[FM:FH], wd_v[FH + FM:]).T
        wo = _quads(_cols(*[wo_t[i] for i in range(NQ)]))
        wo = [_left(i, *wo) for i in range(7)]
        pending = [(j, c) for j in range(NQ) for c in range(NC)]
        last, top, m = {}, {}, {}
        early = 28
        job = second_norm(x1_first, attempt >> 8)

        def last_head(n):
            while len(pending) > max(NQ * NC - n, 0):
                j, c = pending.pop(0)
                pv = _dot(_unpack(v_t[c, (D - DH) // 2:]), p_v[j, c * CK:(c + 1) * CK])
                last[j] = last[j] + pv if c else pv

        def heads(b, lo, hi):
            inv = 1.0 / _rows(*[_row_sums([l_v[b, g + i] for i in range(8)]) for g in range(lo, hi, 8)])
            o = _rows(*[(o_t[b, hd] if hd < H - 1 else last[b]) * inv[hd - lo:hd - lo + 1] for hd in range(lo, hi)])
            return o[:, :BQ // 2], o[:, BQ // 2:]

        for b in range(NQ):
            top[b] = heads(b, 0, H // 2)
            for n, i in enumerate((1, 5)):
                m[b, i] = _dot(wo[i], _right(i, *top[b], None, None))
                last_head((2 * b + n + 1) * early // (2 * NQ))
        for b in range(NQ):
            last_head((b + 1) * NC)
            o = top[b] + heads(b, H // 2, H)
            for n, i in enumerate((3, 0, 2, 4, 6)):
                m[b, i] = _dot(wo[i], _right(i, *o))
                last_head(early + b * NC + (n + 1) * NC // 5)
                if b > 0:
                    advance(job, x1_first, 1, m[b, i][:D // 4])
                    advance(job, x1_first, 1, m[b, i])
            x1 = x_v[b * BQ:(b + 1) * BQ].T.astype(F32) + wide(0) * _join(*_gather([m[b, i] for i in range(7)]))
            x1_v[b] = x1
            if b == 0:
                x1_first[0] = x1
        for _ in job:
            pass
        jax.lax.fori_loop(0, NQ, ffn, None)

        parts = l_v[...].reshape(NQ * H, 8, BQ)
        safe = (jnp.min(parts, axis=0) >= L_MIN) & (jnp.sum(parts, axis=0) <= L_MAX)
        redo = (jnp.max(jnp.where(safe, 0.0, 1.0)) > 0.0) & (attempt == 0)
        for b in range(NQ):
            cp_out(b).wait()

        @pl.when(redo)
        def _():
            jax.lax.fori_loop(0, H * NQ, head_with_true_max, None)

        return jnp.where(redo, 1, 2)

    jax.lax.while_loop(lambda attempt: attempt < 2, finish, 0)


@jax.jit
def pallas_adaLN_cond__mha_block__geglu_ffn__prompt_kernel(
    A_x: jax.Array,
    A_wqkv: jax.Array,
    A_wo: jax.Array,
    B_x: jax.Array,
    B_w_gate: jax.Array,
    B_w_up: jax.Array,
    B_w_down: jax.Array,
    c: jax.Array,
    w_mod: jax.Array,
):
    del B_x
    _, S, D = A_x.shape
    F = B_w_gate.shape[1]
    DH, NQ, NC = D // H, S // BQ, S // CK
    tiles = [2 * (NQ * RB + NC) * DH // NCH + 4] * NCH
    tiles[0] += H * NQ * RB
    tiles[-1] += D // 8 * NC
    hbm = pl.BlockSpec(memory_space=pltpu.HBM)
    out = pl.pallas_call(
        _kernel,
        out_shape=jax.ShapeDtypeStruct((S, D), A_x.dtype),
        in_specs=[hbm] * 8,
        out_specs=hbm,
        scratch_shapes=[
            pltpu.VMEM((S, D), BF16),
            pltpu.VMEM((D, 3 * D), BF16),
            pltpu.VMEM((D, D), BF16),
            pltpu.VMEM((F, D), BF16),
            pltpu.VMEM((F, D), BF16),
            pltpu.VMEM((F, D), BF16),
            pltpu.VMEM((D, 6 * D), BF16),
            pltpu.VMEM((12, F // 4, D // 2), U32),
            pltpu.VMEM((NQ, D, LANES), BF16),
            pltpu.VMEM((F // 256, 7, D // 4, LANES), U32),
            pltpu.VMEM((D, F % 256), BF16),
            pltpu.VMEM((4, D, LANES), F32),
            pltpu.VMEM((NQ, D // 2, BQ), U32),
            pltpu.VMEM((H, S // 2, LANES), U32),
            pltpu.VMEM((NC, D // 2, CK), U32),
            pltpu.VMEM((NQ, H, DH, BQ), F32),
            pltpu.VMEM((NQ, S, BQ), F32),
            pltpu.VMEM((NQ, H, 8, BQ), F32),
            pltpu.VMEM((NQ + 2, D, BQ), F32),
            pltpu.VMEM((2, D, BQ), F32),
            pltpu.VMEM((NQ, BQ, D), BF16),
            pltpu.SemaphoreType.DMA((10 + NQ,)),
            pltpu.SemaphoreType.DMA((NQ,)),
            *[pltpu.VMEM((n, 8, LANES), F32) for n in tiles],
            pltpu.VMEM(c.shape, BF16),
        ],
        compiler_params=pltpu.CompilerParams(vmem_limit_bytes=120 * 1024 * 1024),
        name="adaln_block",
    )(c, A_x.reshape(S, D), A_wqkv, A_wo, B_w_gate.T, B_w_up.T, B_w_down, w_mod)
    return out.reshape(A_x.shape)
```
